```python
import jax
import jax.numpy as jnp

def _softmax(x, axis=-1):
    return jax.nn.softmax(x, axis=axis)

def _gelu(x):
    return jax.nn.gelu(x, approximate=True)

def _silu(x):
    return jax.nn.silu(x)

def _sigmoid(x):
    return jax.nn.sigmoid(x)

def _layernorm(x, axis=-1, eps=1e-05):
    m = jnp.mean(x, axis=axis, keepdims=True)
    v = jnp.var(x, axis=axis, keepdims=True)
    return (x - m) / jnp.sqrt(v + eps)

def _scatter_add(tgt, idx, src, axis=0):
    return tgt.at[idx].add(src)

def _segment_sum(src, seg, n):
    return jax.ops.segment_sum(src, seg, n)

class _Rng:

    def __init__(self, key):
        self._k = key

    def _next(self):
        self._k, sub = jax.random.split(self._k)
        return sub

    def normal(self, shape):
        return jax.random.normal(self._next(), shape, dtype=jnp.bfloat16)

    def randint(self, lo, hi, shape):
        return jax.random.randint(self._next(), shape, lo, hi, dtype=jnp.int32)

    def uniform(self, shape, lo=0.0, hi=1.0):
        return jax.random.uniform(self._next(), shape, jnp.bfloat16, lo, hi)

    def permutation(self, n):
        return jax.random.permutation(self._next(), n)
kernel_name = 'adaLN_cond__sliding_block_cached__mixer_token_mlp__decode'

def setup_inputs():
    _rng = _Rng(jax.random.key(int.from_bytes(__import__("os").urandom(4), "little")))
    _w = lambda a: (lambda t: t.astype(jnp.bfloat16) if jnp.issubdtype(t.dtype, jnp.floating) else t)(jnp.asarray(a))

    def _A_setup():
        B, Sq, D = (1, 1, 640)
        Hq, Hkv, Sk, Dh = (32, 32, 32768, 192)
        assert Hq % Hkv == 0, (Hq, Hkv)
        return {'x': _w((lambda *s: _rng.normal(s) * 0.05)(B, Sq, D)), 'k_cache': _w((lambda *s: _rng.normal(s) * 0.05)(B, Hkv, Sk, Dh)), 'v_cache': _w((lambda *s: _rng.normal(s) * 0.05)(B, Hkv, Sk, Dh)), 'wq': _w((lambda *s: _rng.normal(s) * 0.05)(D, Hq * Dh) * D ** (-0.5)), 'wo': _w((lambda *s: _rng.normal(s) * 0.05)(Hq * Dh, D) * (Hq * Dh) ** (-0.5))}
    _A_in = _A_setup()

    def _B_setup():
        B, S, D, F = (1, 1, 640, 1536)
        return {'x': _w((lambda *s: _rng.normal(s) * 0.05)(B, S, D)), 'w1': _w((lambda *s: _rng.normal(s) * 0.05)(S, F) * S ** (-0.5)), 'b1': _w((lambda *s: _rng.normal(s) * 0.05)(F) * 0.02), 'w2': _w((lambda *s: _rng.normal(s) * 0.05)(F, S) * F ** (-0.5)), 'b2': _w((lambda *s: _rng.normal(s) * 0.05)(S) * 0.02)}
    _B_in = _B_setup()
    return {'A_x': _A_in['x'], 'A_k_cache': _A_in['k_cache'], 'A_v_cache': _A_in['v_cache'], 'A_wq': _A_in['wq'], 'A_wo': _A_in['wo'], 'B_x': _B_in['x'], 'B_w1': _B_in['w1'], 'B_b1': _B_in['b1'], 'B_w2': _B_in['w2'], 'B_b2': _B_in['b2'], 'c': _w((lambda *s: _rng.normal(s) * 0.05)(1, 640)), 'w_mod': _w((lambda *s: _rng.normal(s) * 0.05)(640, 6 * 640) * 640 ** (-0.5))}

def reference(A_x, A_k_cache, A_v_cache, A_wq, A_wo, B_x, B_w1, B_b1, B_w2, B_b2, c, w_mod):

    def _A_ref(x, k_cache, v_cache, wq, wo):
        B, Sq, D = x.shape
        Hq, Dh = (32, 192)
        Hkv, Sk = (k_cache.shape[1], k_cache.shape[2])
        W = min(4096, max(256, Sk // 4))
        rep = Hq // Hkv
        q = (lambda x, *d: x.transpose(*d))((x @ wq).reshape(B, Sq, Hq, Dh), 0, 2, 1, 3)
        k = jnp.repeat(k_cache[:, :, Sk - W:, :], rep, axis=1)
        v = jnp.repeat(v_cache[:, :, Sk - W:, :], rep, axis=1)
        scores = jnp.einsum('bhqd,bhkd->bhqk', q, k) * Dh ** (-0.5)
        p = _softmax(scores, axis=-1)
        o = jnp.einsum('bhqk,bhkd->bhqd', p, v)
        return (lambda x, *d: x.transpose(*d))(o, 0, 2, 1, 3).reshape(B, Sq, Hq * Dh) @ wo

    def _B_ref(x, w1, b1, w2, b2):
        B, S, D = x.shape
        h = _layernorm(x, axis=-1)
        u = jnp.einsum('bsd,sf->bdf', h, w1) + b1
        u = _gelu(u)
        y = jnp.einsum('bdf,fs->bds', u, w2) + b2
        return (lambda x, *d: x.transpose(*d))(y, 0, 2, 1)
    x = A_x
    mod = (_silu(c) @ w_mod).reshape(c.shape[0], 6, 1, -1)
    sa, ca, ga, sb, cb, gb = (mod[:, 0].copy(), mod[:, 1].copy(), mod[:, 2].copy(), mod[:, 3].copy(), mod[:, 4].copy(), mod[:, 5].copy())
    h = _layernorm(x, axis=-1) * (1 + ca) + sa
    x = x + ga * _A_ref(h, A_k_cache, A_v_cache, A_wq, A_wo)
    h = _layernorm(x, axis=-1) * (1 + cb) + sb
    x = x + gb * _B_ref(h, B_w1, B_b1, B_w2, B_b2)
    return x
```

```python
import functools

import jax
import jax.numpy as jnp
from jax import lax
import jax.experimental.pallas as pl
import jax.experimental.pallas.tpu as pltpu


D = 640
H = 32
DH = 192
SK = 32768
W = min(4096, max(256, SK // 4))
F = 1536
PAIR = 2 * DH
NB = 2
NWO = 8
NS = 5
FC = 128
GAT = 10

C1 = 0.7978845608028654
C2 = C1 * 0.044715
S = C2 ** (1.0 / 3.0)
KK = C1 / S


def _ln(x):
    m = jnp.mean(x, axis=-1, keepdims=True)
    xc = x - m
    v = jnp.mean(xc * xc, axis=-1, keepdims=True)
    return xc * lax.rsqrt(v + 1e-5)


def _dot(a, b):
    return jnp.dot(a, b, preferred_element_type=jnp.float32)


def _body(x_hbm, kt, vt, wq_hbm, wo_hbm, w1_hbm, b1_hbm, w2_hbm, b2_hbm, c_hbm, wm_hbm,
          out_ref,
          kbuf, vbuf, wq_v, wo_v, wm_v, x_v, c_v, w1_v, b1_v, w2_v, b2_v, q_s, w1b, b1b,
          ksem, vsem, sem, wosem, ssem):
    f32, bf16 = jnp.float32, jnp.bfloat16
    copy = pltpu.make_async_copy

    def kcp(h, slot):
        return copy(kt.at[0, h, :, pl.ds(SK - W, W)], kbuf.at[slot], ksem.at[slot])

    def vcp(h, slot):
        return copy(vt.at[0, h, :, pl.ds(SK - W, W)], vbuf.at[slot], vsem.at[slot])

    def wmcp(r0, nr, c0, nc, s):
        idx = (pl.ds(r0, nr), pl.ds(c0, nc))
        return copy(wm_hbm.at[idx], wm_v.at[idx], s)

    WOC, SR = H * DH // NWO, D // NS
    c_cp = copy(c_hbm, c_v, sem.at[0])
    x_cp = copy(x_hbm.at[0], x_v, sem.at[1])
    wm1_cp = wmcp(0, D, 0, 2 * D, sem.at[2])
    wq_cp = copy(wq_hbm, wq_v, sem.at[3])
    small = [copy(w1_hbm, w1_v, sem.at[4]), copy(b1_hbm, b1_v, sem.at[5]),
             copy(w2_hbm, w2_v, sem.at[6]), copy(b2_hbm, b2_v, sem.at[7])]
    tail = [copy(wo_hbm.at[pl.ds(i * WOC, WOC)], wo_v.at[pl.ds(i * WOC, WOC)], wosem.at[i])
            for i in range(NWO)]
    tail += [wmcp(0, D, 2 * D, D, sem.at[8])]
    tail += [wmcp(i * SR, SR, 3 * D, 2 * D, ssem.at[i]) for i in range(NS)]
    tail += [wmcp(0, D, 5 * D, D, sem.at[9])]
    pos = [0]

    def start_next_tail():
        if pos[0] < len(tail):
            tail[pos[0]].start()
            pos[0] += 1

    def wait_tail(i):
        tail[i].wait()
        start_next_tail()

    wm1_cp.start()
    c_cp.start()
    x_cp.start()
    wq_cp.start()
    for cp in small:
        cp.start()
    for h in range(NB):
        kcp(h, h).start()
        vcp(h, h).start()

    c_cp.wait()
    x_cp.wait()
    wm1_cp.wait()
    cf = c_v[...].astype(f32)
    sc8 = jnp.broadcast_to((cf * jax.nn.sigmoid(cf)).astype(bf16), (8, D))
    mod1 = _dot(sc8, wm_v[:, 0:2 * D])
    x0 = jnp.broadcast_to(x_v[...].astype(f32), (8, D))
    h1 = _ln(x0) * (1.0 + mod1[:, D:2 * D]) + mod1[:, 0:D]

    for cp in small:
        cp.wait()
    w1r = w1_v[...].astype(f32) * S
    b1r = b1_v[...].astype(f32).reshape(1, F) * S
    w2r = w2_v[...].astype(f32) * (0.5 / S)
    w1b[...] = jnp.broadcast_to(w1r, (128, F)).T
    b1b[...] = jnp.broadcast_to(b1r, (128, F)).T
    lin_a = jnp.sum(w1r * w2r, axis=-1, keepdims=True)
    lin_b = jnp.sum(b1r * w2r, axis=-1, keepdims=True) + b2_v[...].astype(f32).reshape(1, 1)

    wq_cp.wait()
    q = _dot(h1.astype(bf16), wq_v[...])
    for j in range(H // 2):
        q_s[j] = q[:, j * PAIR:(j + 1) * PAIR]

    def pair(j, carry, prefetch):
        qp = q_s[j]
        for t in range(2):
            h = 2 * j + t
            slot = h % NB
            qh = qp[:, t * DH:(t + 1) * DH].astype(bf16)
            kcp(h, slot).wait()
            s = _dot(qh, kbuf[slot]) * (DH ** -0.5)
            if prefetch:
                kcp(h + NB, slot).start()
            else:
                start_next_tail()
            m = jnp.max(s, axis=-1, keepdims=True)
            p = jnp.exp(s - m)
            l = jnp.sum(p, axis=-1, keepdims=True)
            vcp(h, slot).wait()
            o = lax.dot_general(p.astype(bf16), vbuf[slot], (((1,), (1,)), ((), ())),
                                preferred_element_type=f32)
            if prefetch:
                vcp(h + NB, slot).start()
            else:
                start_next_tail()
            q_s[j, :, t * DH:(t + 1) * DH] = o / l
        return carry

    NP = (H - NB) // 2
    lax.fori_loop(0, NP, functools.partial(pair, prefetch=True), 0)
    for j in range(NP, H // 2):
        pair(j, 0, False)

    acc = jnp.zeros((8, D), f32)
    ppc = WOC // PAIR
    for i in range(NWO):
        wait_tail(i)
        for j in range(i * ppc, (i + 1) * ppc):
            acc += _dot(q_s[j].astype(bf16), wo_v[j * PAIR:(j + 1) * PAIR, :])
    wait_tail(NWO)
    ga = _dot(sc8, wm_v[:, 2 * D:3 * D])
    x1 = x0 + ga * acc
    n1 = _ln(x1)
    mod2 = jnp.zeros((8, 2 * D), f32)
    for i in range(NS):
        wait_tail(NWO + 1 + i)
        mod2 += _dot(sc8[:, i * SR:(i + 1) * SR], wm_v[i * SR:(i + 1) * SR, 3 * D:5 * D])
    h2 = _ln(n1 * (1.0 + mod2[:, D:]) + mod2[:, :D])[0:1]

    w2bf = jnp.broadcast_to(w2_v[...], (8, F))
    y = jnp.zeros((8, D), f32)
    gb = None
    for i in range(F // FC):
        if i == GAT:
            wait_tail(NWO + 1 + NS)
            gb = _dot(sc8, wm_v[:, 5 * D:6 * D])
        a = w1b[i * FC:(i + 1) * FC, :]
        b = b1b[i * FC:(i + 1) * FC, :]
        ps = []
        for t in range(D // 128):
            z = h2[:, t * 128:(t + 1) * 128] * a + b
            ps.append(z * jnp.tanh(z * (z * z + KK)))
        y += _dot(w2bf[:, i * FC:(i + 1) * FC], jnp.concatenate(ps, axis=1).astype(bf16))
    y = y[0:1] * (0.5 / S) + (h2 * lin_a + lin_b)
    out_ref[0] = (x1[0:1] + gb[0:1] * y).astype(out_ref.dtype)


@jax.jit
def pallas_adaLN_cond__sliding_block_cached__mixer_token_mlp__decode_kernel(
    A_x: jax.Array,
    A_k_cache: jax.Array,
    A_v_cache: jax.Array,
    A_wq: jax.Array,
    A_wo: jax.Array,
    B_x: jax.Array,
    B_w1: jax.Array,
    B_b1: jax.Array,
    B_w2: jax.Array,
    B_b2: jax.Array,
    c: jax.Array,
    w_mod: jax.Array,
):
    kt = jnp.swapaxes(A_k_cache, 2, 3)
    vt = jnp.swapaxes(A_v_cache, 2, 3)
    bf, f32 = jnp.bfloat16, jnp.float32
    DMA = pltpu.SemaphoreType.DMA
    return pl.pallas_call(
        _body,
        out_shape=jax.ShapeDtypeStruct((1, 1, D), A_x.dtype),
        in_specs=[pl.BlockSpec(memory_space=pl.ANY)] * 11,
        out_specs=pl.BlockSpec(memory_space=pltpu.VMEM),
        scratch_shapes=[
            pltpu.VMEM((NB, DH, W), bf), pltpu.VMEM((NB, DH, W), bf),
            pltpu.VMEM((D, H * DH), bf), pltpu.VMEM((H * DH, D), bf), pltpu.VMEM((D, 6 * D), bf),
            pltpu.VMEM((1, D), bf), pltpu.VMEM((1, D), bf),
            pltpu.VMEM((1, F), bf), pltpu.VMEM((F,), bf), pltpu.VMEM((1, F), bf), pltpu.VMEM((1,), bf),
            pltpu.VMEM((H // 2, 8, PAIR), f32),
            pltpu.VMEM((F, 128), f32), pltpu.VMEM((F, 128), f32),
            DMA((NB,)), DMA((NB,)), DMA((10,)), DMA((NWO,)), DMA((NS,)),
        ],
        compiler_params=pltpu.CompilerParams(vmem_limit_bytes=64 * 1024 * 1024),
    )(A_x, kt, vt, A_wq, A_wo, B_w1, B_b1, B_w2.T, B_b2, c, w_mod)
```
